```python
import jax
import jax.numpy as jnp

def _softmax(x, axis=-1):
    return jax.nn.softmax(x, axis=axis)
def _gelu(x):
    return jax.nn.gelu(x, approximate=True)
def _silu(x):
    return jax.nn.silu(x)
def _sigmoid(x):
    return jax.nn.sigmoid(x)
def _layernorm(x, axis=-1, eps=1e-5):
    m = jnp.mean(x, axis=axis, keepdims=True)
    v = jnp.var(x, axis=axis, keepdims=True)
    return (x - m) / jnp.sqrt(v + eps)
def _scatter_add(tgt, idx, src, axis=0):
    return tgt.at[idx].add(src)
def _segment_sum(src, seg, n):
    return jax.ops.segment_sum(src, seg, n)
class _Rng:
    def __init__(self, key):
        self._k = key
    def _next(self):
        self._k, sub = jax.random.split(self._k)
        return sub
    def normal(self, shape):
        return jax.random.normal(self._next(), shape, dtype=jnp.bfloat16)
    def randint(self, lo, hi, shape):
        return jax.random.randint(self._next(), shape, lo, hi, dtype=jnp.int32)
    def uniform(self, shape, lo=0.0, hi=1.0):
        return jax.random.uniform(self._next(), shape, jnp.bfloat16, lo, hi)
    def permutation(self, n):
        return jax.random.permutation(self._next(), n)


kernel_name = 'interleave_layers__linear_kernel_hedgehog__sliding_local_dilated__prompt'

def setup_inputs():
    _rng = _Rng(jax.random.key(int.from_bytes(__import__("os").urandom(4), "little")))
    _w = (lambda a: (lambda t: t.astype(jnp.bfloat16) if jnp.issubdtype(t.dtype, jnp.floating) else t)(jnp.asarray(a)))
    def _A_setup():
        B, S, D, H = 1, 2048, 1024, 32
        Dh = D // H
        return {
            "x": _w((lambda *s: _rng.normal(s) * 0.05)(B, S, D)),
            "wqkv": _w((lambda *s: _rng.normal(s) * 0.05)(D, 3 * D)),
            "w_phi": _w((lambda *s: _rng.normal(s) * 0.05)(H, Dh, Dh) * (Dh ** -0.5)),
            "wo": _w((lambda *s: _rng.normal(s) * 0.05)(D, D)),
        }
    _A_in = _A_setup()

    def _B_setup():
        B, S, D = 1, 2048, 1024
        return {
            "x": _w((lambda *s: _rng.normal(s) * 0.05)(B, S, D)),
            "wqkv": _w((lambda *s: _rng.normal(s) * 0.05)(D, 3 * D)),
            "wo": _w((lambda *s: _rng.normal(s) * 0.05)(D, D)),
        }
    _B_in = _B_setup()

    return {
        "A_x": _A_in["x"],
        "A_wqkv": _A_in["wqkv"],
        "A_w_phi": _A_in["w_phi"],
        "A_wo": _A_in["wo"],
        "B_x": _B_in["x"],
        "B_wqkv": _B_in["wqkv"],
        "B_wo": _B_in["wo"],
    }

def reference(A_x, A_wqkv, A_w_phi, A_wo, B_x, B_wqkv, B_wo):
    def _A_ref(x, wqkv, w_phi, wo):
        B, S, D = x.shape
        H = 32; Dh = D // H
        qkv = (lambda x, *d: x.transpose(*d))((x @ wqkv).reshape(B, S, 3, H, Dh), 2, 0, 3, 1, 4)
        q, k, v = qkv[0], qkv[1], qkv[2]
        pq = jnp.einsum("bhsd,hdf->bhsf", q, w_phi)
        pk = jnp.einsum("bhsd,hdf->bhsf", k, w_phi)
        phi_q = jnp.concatenate([_softmax(pq, axis=-1), _softmax(-pq, axis=-1)], axis=-1)
        phi_k = jnp.concatenate([_softmax(pk, axis=-1), _softmax(-pk, axis=-1)], axis=-1)
        kv = jnp.einsum("bhsf,bhsd->bhfd", phi_k, v)
        z  = jnp.einsum("bhsf->bhf", phi_k)
        num = jnp.einsum("bhqf,bhfd->bhqd", phi_q, kv)
        den = jnp.einsum("bhqf,bhf->bhq", phi_q, z)[..., None] + 1e-6
        o = num / den
        return (lambda x, *d: x.transpose(*d))(o, 0, 2, 1, 3).reshape(B, S, D) @ wo

    def _B_ref(x, wqkv, wo):
        B, S, D = x.shape
        H = 32; Dh = D // H
        W, dil = 8, 2
        qkv = (lambda x, *d: x.transpose(*d))((x @ wqkv).reshape(B, S, 3, H, Dh), 2, 0, 3, 1, 4)
        q, k, v = qkv[0], qkv[1], qkv[2]
        scale = Dh ** -0.5
        pos = jnp.arange(S)
        off = jnp.arange(W) * dil
        idx = pos[:, None] - off[None, :]
        mask = idx >= 0
        idx_c = jnp.where(mask, idx, 0).reshape(-1)
        kg = k[:, :, idx_c, :].reshape(B, H, S, W, Dh)
        vg = v[:, :, idx_c, :].reshape(B, H, S, W, Dh)
        logits = jnp.einsum("bhsd,bhswd->bhsw", q, kg) * scale
        logits = jnp.where(mask[None, None, :, :], logits, -1e9)
        attn = _softmax(logits, axis=-1)
        o = jnp.einsum("bhsw,bhswd->bhsd", attn, vg)
        return (lambda x, *d: x.transpose(*d))(o, 0, 2, 1, 3).reshape(B, S, D) @ wo

    x = A_x
    x = x + _A_ref(_layernorm(x, axis=-1), A_wqkv, A_w_phi, A_wo)
    x = x + _B_ref(_layernorm(x, axis=-1), B_wqkv, B_wo)
    x = x + _A_ref(_layernorm(x, axis=-1), A_wqkv, A_w_phi, A_wo)
    x = x + _B_ref(_layernorm(x, axis=-1), B_wqkv, B_wo)
    return x
```

```python
import functools
import numpy as np
import jax
import jax.numpy as jnp
from jax import lax
from jax.experimental import pallas as pl
from jax.experimental.pallas import tpu as pltpu

S, D, H, DH = 2048, 1024, 32, 32
NC = 16
L = 128
GA = 4
NGA = H // GA
RA = GA * DH
GB = 8
NGB = H // GB
RB = GB * DH
CT = 2
NT = CT * L
NJ = NC // CT
W_WIN = 8
LOG2E = 1.4426950408889634
EPS = 1e-5
MC = 128
f32, bf16, u32 = jnp.float32, jnp.bfloat16, jnp.uint32
NT_DIMS = (((1,), (1,)), ((), ()))


def _sigma(k):
    return 16 * (k // 16) + 8 * (k % 2) + (k % 16) // 2


def _consts():
    def c_of_r(r):
        p, rr = r // 64, r % 64
        return p * 64 + (rr % 2) * 32 + rr // 2
    perm_v = np.zeros((RA, RA), np.float32)
    emat = np.zeros((RA, DH), np.float32)
    bdm = np.zeros((RA, RA), np.float32)
    perm_o = np.zeros((RA, RA), np.float32)
    for r in range(RA):
        c = c_of_r(r)
        perm_v[r, c] = 1
        emat[r, (r % 64) // 2] = 1
        bdm[r, (c // 32) * 32:(c // 32) * 32 + 32] = 1
    for k2 in range(RA):
        o_row = _sigma(k2)
        p, k = o_row // 64, o_row % 64
        perm_o[k2, c_of_r(p * 64 + _sigma(k))] = 1
    out = np.zeros((3 * RA, RA), np.float32)
    out[0:RA] = perm_v
    out[RA:2 * RA] = bdm
    out[2 * RA:] = perm_o
    return out


def pk(x):
    return pltpu.bitcast(x.astype(bf16), u32)


def pkf(x):
    n, m = x.shape[0] // 16, x.shape[1]
    x4 = x.reshape(n, 2, 8, m)
    return pltpu.pack_elementwise([x4[:, 0], x4[:, 1]], packed_dtype=bf16).reshape(8 * n, m)


def upk(x):
    return pltpu.bitcast(x, bf16)


def _rcp(x):
    return pl.reciprocal(x, approx=True)


def _par_all(x, op):
    x = op(x, pltpu.roll(x, 2, 0))
    return op(x, pltpu.roll(x, 4, 0))


def _sub_all(x):
    x = x + pltpu.roll(x, 1, 0)
    x = x + pltpu.roll(x, 2, 0)
    return x + pltpu.roll(x, 4, 0)


def _phi_pair(p):
    n = p.shape[1]
    p3 = p.reshape(8, 8, n)
    mx = _par_all(jnp.max(p3, axis=0), jnp.maximum)
    mn = _par_all(jnp.min(p3, axis=0), jnp.minimum)
    e1 = jnp.exp2(p3 - mx[None])
    e2 = jnp.exp2(mn[None] - p3)
    r1 = _rcp(_par_all(jnp.sum(e1, axis=0), jnp.add))
    r2 = _rcp(_par_all(jnp.sum(e2, axis=0), jnp.add))
    a = (e1 * r1[None]).reshape(2 * DH, n)
    b = (e2 * r2[None]).reshape(2 * DH, n)
    return jnp.concatenate([a, b], axis=0).astype(bf16)


def _ln_finish(xT_s, hT_s, jp, ssum):
    m = _sub_all(ssum) * (1.0 / D)
    acc = None
    for c in range(D // MC):
        d = xT_s[jp, c * MC:(c + 1) * MC, :].reshape(MC // 8, 8, NT) - m[None]
        t = jnp.sum(d * d, axis=0)
        acc = t if acc is None else acc + t
    r = lax.rsqrt(_sub_all(acc) * (1.0 / D) + EPS)
    for c in range(D // MC):
        d = xT_s[jp, c * MC:(c + 1) * MC, :].reshape(MC // 8, 8, NT) - m[None]
        hT_s[jp, c * (MC // 2):(c + 1) * (MC // 2), :] = pkf((d * r[None]).reshape(MC, NT))


def kernel(x_ref, awqkv_ref, awphi_ref, awo_ref, bwqkv_ref, bwo_ref, cst_ref, o_ref,
           xf_s, xT_s, hT_s, oT_s, waq_s, wakv_s, wbq_s, wbkv_s, woa_s, wob_s,
           q_s, k_s, v_s, vb_s, kvacc_s, kvT_s, tmp_s, tmpu_s):
    with jax.named_scope("wprep"):
        perm_v = cst_ref[0:RA, :]
        bdm = cst_ref[RA:2 * RA, :]
        perm_o = cst_ref[2 * RA:3 * RA, :]
        e_r = lax.broadcasted_iota(jnp.int32, (RA, DH), 0)
        e_f = lax.broadcasted_iota(jnp.int32, (RA, DH), 1)
        emat = jnp.where((e_r % 64) // 2 == e_f, 1.0, 0.0).astype(bf16)

        def kperm(w):
            return upk(pkf(w.astype(f32)))

        for g in range(NGA):
            cs = slice(g * RA, (g + 1) * RA)
            wp = awphi_ref[cs, :]
            bdT = lax.dot_general(emat, wp, NT_DIMS, preferred_element_type=f32)
            bdT = (bdT * bdm.astype(f32)).astype(bf16)
            for it in range(D // 256):
                rs = slice(it * 256, (it + 1) * 256)
                wq = lax.dot_general(bdT, kperm(awqkv_ref[rs, g * RA:(g + 1) * RA]), NT_DIMS, preferred_element_type=f32)
                waq_s[g, :, rs] = pk(wq * LOG2E)
                wk = lax.dot_general(bdT, kperm(awqkv_ref[rs, D + g * RA:D + (g + 1) * RA]), NT_DIMS, preferred_element_type=f32)
                wakv_s[g, 0:RA // 2, rs] = pk(wk * LOG2E)
                wv = lax.dot_general(perm_v, kperm(awqkv_ref[rs, 2 * D + g * RA:2 * D + (g + 1) * RA]), NT_DIMS, preferred_element_type=f32)
                wakv_s[g, RA // 2:RA, rs] = pk(wv)
            for ot in range(D // L):
                wo_p = jnp.dot(perm_o, awo_ref[cs, ot * L:(ot + 1) * L], preferred_element_type=f32)
                woa_s[ot * (L // 2):(ot + 1) * (L // 2), cs] = pk(wo_p.T)
        for g in range(NGB):
            for part in range(3):
                c0 = part * D + g * RB
                for it in range(D // L):
                    blk = kperm(bwqkv_ref[it * L:(it + 1) * L, c0:c0 + RB]).astype(f32)
                    tmp_s[0:L, :] = blk[:, 0:L].T
                    tmp_s[L:2 * L, :] = blk[:, L:2 * L].T
                    rows = [tmp_s[pl.ds(d, 8, stride=DH), :] for d in range(DH)]
                    wt = pk(jnp.concatenate(rows, axis=0))
                    if part == 0:
                        wbq_s[g, :, it * L:(it + 1) * L] = wt
                    else:
                        wbkv_s[g, (part - 1) * (RB // 2):part * (RB // 2), it * L:(it + 1) * L] = wt
            for ot in range(D // L):
                tmpu_s[...] = pltpu.bitcast(bwo_ref[g * RB:(g + 1) * RB, ot * L:(ot + 1) * L], u32)
                rows = [tmpu_s[pl.ds(t, 8, stride=16), :] for t in range(16)]
                wr = upk(jnp.concatenate(rows, axis=0)).astype(f32)
                wob_s[ot * (L // 2):(ot + 1) * (L // 2), g * RB:g * RB + L] = pk(wr[0:L].T)
                wob_s[ot * (L // 2):(ot + 1) * (L // 2), g * RB + L:(g + 1) * RB] = pk(wr[L:2 * L].T)

    with jax.named_scope("xprep"):
        for dt in range(D // L):
            xf_s[dt] = x_ref[:, dt * L:(dt + 1) * L].astype(f32)
        for j in range(NC):
            for dt in range(D // L):
                xc = xf_s[dt, pl.ds(j, L, stride=NC), :]
                xT_s[j // CT, dt * L:(dt + 1) * L, (j % CT) * L:(j % CT + 1) * L] = xc.T
        for jp in range(NJ):
            ssum = None
            for c in range(D // MC):
                t = jnp.sum(xT_s[jp, c * MC:(c + 1) * MC, :].reshape(MC // 8, 8, NT), axis=0)
                ssum = t if ssum is None else ssum + t
            _ln_finish(xT_s, hT_s, jp, ssum)

    kr = lax.broadcasted_iota(jnp.int32, (2 * DH, L), 0)
    kc = lax.broadcasted_iota(jnp.int32, (2 * DH, L), 1)
    par_mask = ((kr // 2) % 2) == (kc % 2)
    zr = lax.broadcasted_iota(jnp.int32, (16, L), 0)
    z_mask = (((zr // 2) % 2) == (lax.broadcasted_iota(jnp.int32, (16, L), 1) % 2)) & (zr < 8)

    def a_mm_kv(g, jp):
        r = jnp.dot(upk(wakv_s[g]), upk(hT_s[jp]), preferred_element_type=f32)
        buf = g % 2
        k_s[buf, jp, 0:RA, :] = r[0:RA]
        vb_s[buf, jp] = pkf(r[RA:2 * RA])

    def a_mm_q(g, jp):
        q_s[jp, 0:RA, :] = jnp.dot(upk(waq_s[g]), upk(hT_s[jp]), preferred_element_type=f32)

    def a_phik(g, jp):
        buf = g % 2
        for p in range(GA // 2):
            phi = _phi_pair(k_s[buf, jp, p * 64:(p + 1) * 64, :])
            vv = upk(vb_s[buf, jp, p * DH:(p + 1) * DH, :])
            vaug = jnp.concatenate([vv, jnp.ones((16, NT), bf16)], axis=0)
            kv = lax.dot_general(vaug, phi, NT_DIMS, preferred_element_type=f32)
            if jp == 0:
                kvacc_s[p] = kv
            else:
                kvacc_s[p] += kv

    def a_fin():
        for p in range(GA // 2):
            a = jnp.where(par_mask, kvacc_s[p, 0:2 * DH, :], 0.0)
            b = jnp.where(z_mask, kvacc_s[p, 2 * DH:, :], 0.0)
            kvT_s[p] = pk(jnp.concatenate([a, b], axis=0))

    def a_out(g, jp):
        for p in range(GA // 2):
            phi = _phi_pair(q_s[jp, p * 64:(p + 1) * 64, :])
            nd = jnp.dot(upk(kvT_s[p]), phi, preferred_element_type=f32)
            rcp = _rcp(nd[2 * DH:2 * DH + 8] + 1e-6)
            o = (nd[0:2 * DH].reshape(8, 8, NT) * rcp[None]).reshape(2 * DH, NT)
            oT_s[jp, pl.ds(pl.multiple_of(g * (RA // 2) + p * DH, DH), DH), :] = pkf(o)

    def layer_a():
        for jp in range(NJ):
            a_mm_kv(0, jp)
        for jp in range(NJ):
            a_mm_kv(1, jp)
            a_phik(0, jp)
        a_mm_q(0, 0)

        def step_body(g, has_kv, last):
            a_fin()
            for jp in range(NJ):
                if has_kv:
                    a_mm_kv(g + 1, jp)
                if jp < NJ - 1:
                    a_mm_q(g - 1, jp + 1)
                elif not last:
                    a_mm_q(g, 0)
                if not last:
                    a_phik(g, jp)
                a_out(g - 1, jp)

        def step(g, c):
            step_body(g, True, False)
            return c
        lax.fori_loop(1, NGA - 1, step, 0)
        step_body(NGA - 1, False, False)
        step_body(NGA, False, True)

    lane0 = lax.broadcasted_iota(jnp.int32, (8, L), 1) == 0
    qscale = (DH ** -0.5) * LOG2E

    def b_mm_kv(g, jp):
        buf = g % 2
        for part, dst in ((0, k_s), (1, v_s)):
            r = jnp.dot(upk(wbkv_s[g, part * (RB // 2):(part + 1) * (RB // 2), :]), upk(hT_s[jp]), preferred_element_type=f32)
            for c in range(CT):
                j = jp * CT + c
                kc = r[:, c * L:(c + 1) * L]
                dst[buf, (NC + j) // CT, :, c * L:(c + 1) * L] = kc
                if j >= 2:
                    dst[buf, jp, :, c * L:(c + 1) * L] = pltpu.roll(kc, 1, 1)

    def b_mm_q(g, jp):
        q_s[jp] = jnp.dot(upk(wbq_s[g]), upk(hT_s[jp]), preferred_element_type=f32) * qscale

    def b_att(g, jp):
        buf = g % 2
        for c in range(CT):
            j = jp * CT + c
            q = q_s[jp, :, c * L:(c + 1) * L].reshape(DH, 8, L)
            ls = []
            for w in range(W_WIN):
                e = j - 2 * w + NC
                kk = k_s[buf, e // CT, :, (e % CT) * L:(e % CT + 1) * L].reshape(DH, 8, L)
                l = jnp.sum(q * kk, axis=0)
                if 2 * w > j:
                    l = jnp.where(lane0, -1e9 * LOG2E, l)
                ls.append(l)
            m = functools.reduce(jnp.maximum, ls)
            es = [jnp.exp2(l - m) for l in ls]
            rcp = _rcp(functools.reduce(lambda a, b: a + b, es))
            acc = None
            for w in range(W_WIN):
                e = j - 2 * w + NC
                vv = v_s[buf, e // CT, :, (e % CT) * L:(e % CT + 1) * L].reshape(DH, 8, L)
                t = vv * (es[w] * rcp)[None]
                acc = t if acc is None else acc + t
            oT_s[jp, pl.ds(pl.multiple_of(g * (RB // 2), RB // 2), RB // 2), c * L:(c + 1) * L] = pkf(acc.reshape(RB, L))

    def layer_b():
        for jp in range(NJ):
            b_mm_kv(0, jp)
        b_mm_q(0, 0)

        def step_body(g, last):
            for jp in range(NJ):
                if not last:
                    b_mm_kv(g + 1, jp)
                if jp < NJ - 1:
                    b_mm_q(g, jp + 1)
                elif not last:
                    b_mm_q(g + 1, 0)
                b_att(g, jp)

        def step(g, c):
            step_body(g, False)
            return c
        lax.fori_loop(0, NGB - 1, step, 0)
        step_body(NGB - 1, True)

    def proj(wo_s, last):
        for jp in range(NJ):
            ssum = None
            for c in range(D // MC):
                rs = slice(c * MC, (c + 1) * MC)
                out = jnp.dot(upk(wo_s[c * (MC // 2):(c + 1) * (MC // 2), :]), upk(oT_s[jp]), preferred_element_type=f32)
                xn = xT_s[jp, rs, :] + out
                if last:
                    for cc in range(CT):
                        j = jp * CT + cc
                        xf_s[c, pl.ds(j, L, stride=NC), :] = xn[:, cc * L:(cc + 1) * L].T
                else:
                    xT_s[jp, rs, :] = xn
                    t = jnp.sum(xn.reshape(MC // 8, 8, NT), axis=0)
                    ssum = t if ssum is None else ssum + t
            if not last:
                _ln_finish(xT_s, hT_s, jp, ssum)

    with jax.named_scope("la0"): layer_a()
    with jax.named_scope("pa0"): proj(woa_s, False)
    with jax.named_scope("lb0"): layer_b()
    with jax.named_scope("pb0"): proj(wob_s, False)
    with jax.named_scope("la1"): layer_a()
    with jax.named_scope("pa1"): proj(woa_s, False)
    with jax.named_scope("lb1"): layer_b()
    with jax.named_scope("pb1"): proj(wob_s, True)
    with jax.named_scope("tail"):
        for dt in range(D // L):
            o_ref[:, dt * L:(dt + 1) * L] = xf_s[dt].astype(bf16)


def build():
    scratch = [
        pltpu.VMEM((D // L, S, L), f32),
        pltpu.VMEM((NJ, D, NT), f32),
        pltpu.VMEM((NJ, D // 2, NT), u32),
        pltpu.VMEM((NJ, D // 2, NT), u32),
        pltpu.VMEM((NGA, RA // 2, D), u32),
        pltpu.VMEM((NGA, RA, D), u32),
        pltpu.VMEM((NGB, RB // 2, D), u32),
        pltpu.VMEM((NGB, RB, D), u32),
        pltpu.VMEM((D // 2, D), u32),
        pltpu.VMEM((D // 2, D), u32),
        pltpu.VMEM((NJ, RB, NT), f32),
        pltpu.VMEM((2, 2 * NJ, RB, NT), f32),
        pltpu.VMEM((2, 2 * NJ, RB, NT), f32),
        pltpu.VMEM((2, NJ, RA // 2, NT), u32),
        pltpu.VMEM((GA // 2, 80, L), f32),
        pltpu.VMEM((GA // 2, 40, L), u32),
        pltpu.VMEM((2 * L, L), f32),
        pltpu.VMEM((L, L), u32),
    ]
    return pl.pallas_call(
        kernel,
        out_shape=jax.ShapeDtypeStruct((S, D), bf16),
        scratch_shapes=scratch,
        compiler_params=pltpu.CompilerParams(vmem_limit_bytes=112 * 1024 * 1024),
    )


@jax.jit
def pallas_interleave_layers__linear_kernel_hedgehog__sliding_local_dilated__prompt_kernel(A_x, A_wqkv, A_w_phi, A_wo, B_x, B_wqkv, B_wo):
    cst = jnp.asarray(_consts(), bf16)
    out = build()(A_x.reshape(S, D), A_wqkv, A_w_phi.reshape(H * DH, DH), A_wo, B_wqkv, B_wo, cst)
    return out.reshape(1, S, D)
```

```python
import functools
import numpy as np
import jax
import jax.numpy as jnp
from jax import lax
from jax.experimental import pallas as pl
from jax.experimental.pallas import tpu as pltpu

S, D, H, DH = 2048, 1024, 32, 32
NC = 16
L = 128
GA = 4
NGA = H // GA
RA = GA * DH
GB = 8
NGB = H // GB
RB = GB * DH
CT = 2
NT = CT * L
NJ = NC // CT
W_WIN = 8
LOG2E = 1.4426950408889634
EPS = 1e-5
KPRE = 256
MC = 128
f32, bf16, u32 = jnp.float32, jnp.bfloat16, jnp.uint32
NT_DIMS = (((1,), (1,)), ((), ()))


def _sigma(k):
    return 16 * (k // 16) + 8 * (k % 2) + (k % 16) // 2


def _consts():
    def c_of_r(r):
        p, rr = r // 64, r % 64
        return p * 64 + (rr % 2) * 32 + rr // 2
    perm_v = np.zeros((RA, RA), np.float32)
    emat = np.zeros((RA, DH), np.float32)
    bdm = np.zeros((RA, RA), np.float32)
    perm_o = np.zeros((RA, RA), np.float32)
    for r in range(RA):
        c = c_of_r(r)
        perm_v[r, c] = 1
        emat[r, (r % 64) // 2] = 1
        bdm[r, (c // 32) * 32:(c // 32) * 32 + 32] = 1
    for k2 in range(RA):
        o_row = _sigma(k2)
        p, k = o_row // 64, o_row % 64
        perm_o[k2, c_of_r(p * 64 + _sigma(k))] = 1
    return np.concatenate([bdm, perm_o, np.ones((16, RA), np.float32)], axis=0)


def pk(x):
    return pltpu.bitcast(x.astype(bf16), u32)


def pkf(x):
    n, m = x.shape[0] // 16, x.shape[1]
    x4 = x.reshape(n, 2, 8, m)
    return pltpu.pack_elementwise([x4[:, 0], x4[:, 1]], packed_dtype=bf16).reshape(8 * n, m)


def upk(x):
    return pltpu.bitcast(x, bf16)


def w_side(a11, a12, a21, a22):
    return [a11 + a22, a21 + a22, a11, a22, a11 + a12, a21 - a11, a12 - a22]


def h_side(b11, b12, b21, b22):
    return [b11 + b22, b11, b12 - b22, b21 - b11, b22, b11 + b12, b21 + b22]


def _rcp(x):
    return pl.reciprocal(x, approx=True)


def _par_all(x, op):
    x = op(x, pltpu.roll(x, 2, 0))
    return op(x, pltpu.roll(x, 4, 0))


def _sub_all(x):
    x = x + pltpu.roll(x, 1, 0)
    x = x + pltpu.roll(x, 2, 0)
    return x + pltpu.roll(x, 4, 0)


def _phi_pair(p):
    n = p.shape[1]
    p3 = p.reshape(8, 8, n)
    mx = _par_all(jnp.max(p3, axis=0), jnp.maximum)
    mn = _par_all(jnp.min(p3, axis=0), jnp.minimum)
    e1 = jnp.exp2(p3 - mx[None])
    e2 = jnp.exp2(mn[None] - p3)
    r1 = _rcp(_par_all(jnp.sum(e1, axis=0), jnp.add))
    r2 = _rcp(_par_all(jnp.sum(e2, axis=0), jnp.add))
    a = (e1 * r1[None]).reshape(2 * DH, n)
    b = (e2 * r2[None]).reshape(2 * DH, n)
    return jnp.concatenate([a, b], axis=0).astype(bf16)


def _ln_finish(xT_s, hT_s, jp, ssum):
    m = _sub_all(ssum) * (1.0 / D)
    acc = None
    for c in range(D // MC):
        d = xT_s[jp, c * MC:(c + 1) * MC, :].reshape(MC // 8, 8, NT) - m[None]
        t = jnp.sum(d * d, axis=0)
        acc = t if acc is None else acc + t
    r = lax.rsqrt(_sub_all(acc) * (1.0 / D) + EPS)
    for c in range(D // 2 // MC):
        t, b = [((xT_s[jp, r0:r0 + MC, :].reshape(MC // 8, 8, NT) - m[None]) * r[None]).reshape(MC, NT)
                for r0 in (c * MC, D // 2 + c * MC)]
        for i, hh in enumerate(h_side(t[:, :L], t[:, L:], b[:, :L], b[:, L:])):
            hT_s[jp, i, c * (MC // 2):(c + 1) * (MC // 2), :] = pkf(hh)


def kernel(x_hbm, awqkv_hbm, wphi_ref, awo_hbm, bwqkv_hbm, bwo_hbm, cst_ref, o_hbm,
           xu_s, sta_s, stb_s, stoa_s, stob_s,
           xT_s, hT_s, oT_s, waq_s, wakv_s, wb_s, woa_s, wob_s, bd_s,
           q_s, k_s, v_s, vb_s, kvacc_s, kvT_s, tmp_s, tmpa_s, tmpu_s,
           sem_x, sem_a, sem_b, sem_oa, sem_ob, sem_o):
    def cp_x(dt):
        return pltpu.make_async_copy(x_hbm.at[:, pl.ds(dt * L, L)], xu_s.at[dt].bitcast(bf16), sem_x.at[0])

    def cp_out(dt):
        return pltpu.make_async_copy(xu_s.at[dt].bitcast(bf16), o_hbm.at[:, pl.ds(dt * L, L)], sem_o.at[0])

    def cp_a(part, g):
        t = g if part > 0 else g + 1
        return pltpu.make_async_copy(awqkv_hbm.at[:, pl.ds(part * D + g * RA, RA)],
                                     sta_s.at[part * NGA + g].bitcast(bf16), sem_a.at[min(t, 3)])

    def cps_a(t):
        return ([cp_a(1, t), cp_a(2, t)] if t < NGA else []) + ([cp_a(0, t - 1)] if t > 0 else [])

    def cp_b(i, half):
        g, part = i // 3, i % 3
        return pltpu.make_async_copy(bwqkv_hbm.at[:, pl.ds(part * D + g * RB + half * L, L)],
                                     stb_s.at[i, half].bitcast(bf16), sem_b.at[i])

    def wait_b(i):
        for half in range(2):
            pltpu.make_async_copy(bwqkv_hbm.at[:, pl.ds(0, L)], stb_s.at[i, half].bitcast(bf16), sem_b.at[i]).wait()

    cp_oa = pltpu.make_async_copy(awo_hbm, stoa_s, sem_oa.at[0])
    cp_ob = pltpu.make_async_copy(bwo_hbm, stob_s, sem_ob.at[0])

    for c in cps_a(0):
        c.start()
    for dt in range(D // L):
        cp_x(dt).start()

    bdm = cst_ref[0:RA, :]
    perm_o = cst_ref[RA:2 * RA, :]
    e_r = lax.broadcasted_iota(jnp.int32, (RA, DH), 0)
    e_f = lax.broadcasted_iota(jnp.int32, (RA, DH), 1)
    emat = jnp.where((e_r % 64) // 2 == e_f, 1.0, 0.0).astype(bf16)

    def kperm(w):
        return upk(pkf(upk(w).astype(f32)))

    pins = []
    always = cst_ref[2 * RA:2 * RA + 16, :].astype(f32)[0:8] > 0.0

    def pin(words):
        pins.append(functools.reduce(jnp.bitwise_or, [words[i:i + 8, j:j + L] for i in range(0, words.shape[0], 8)
                                                      for j in range(0, words.shape[1], L)]))

    def tie(x):
        if not pins:
            return x
        junk = pltpu.bitcast(functools.reduce(jnp.bitwise_or, pins), f32)
        pins.clear()
        return jnp.concatenate([jnp.where(always, x[:, 0:L], junk), x[:, L:]], axis=1)

    late = []

    def done(words):
        words = words if words.dtype == u32 else pltpu.bitcast(words, u32)
        late.append(functools.reduce(jnp.bitwise_or, [words[i:i + 8, j:j + L] for i in range(0, words.shape[0], 8)
                                                      for j in range(0, words.shape[1], L)]))

    def patch(x, pts):
        if not pts:
            return x
        cols = []
        for c in range(x.shape[1] // L):
            rows, r = [], 0
            for (k, cc), junk in sorted(pts.items(), key=lambda kv: kv[0]):
                if cc == c:
                    if k > r:
                        rows.append(x[r:k, c * L:(c + 1) * L])
                    rows.append(jnp.where(always, x[k:k + 8, c * L:(c + 1) * L], junk))
                    r = k + 8
            if r < x.shape[0]:
                rows.append(x[r:, c * L:(c + 1) * L])
            cols.append(jnp.concatenate(rows, axis=0) if len(rows) > 1 else rows[0])
        return jnp.concatenate(cols, axis=1)

    def smm(w, jp, n=0):
        if not TIES:
            late.clear()
        n = min(n, 7, len(late))
        stops = {i * 7 // n: late.pop(0) for i in range(n)}

        def prod(pos, i):
            h = hT_s[jp, i]
            if pos in stops:
                h = patch(h, {(0, 0): stops[pos]})
            return jnp.dot(upk(w[i]), upk(h), preferred_element_type=f32)

        m1, m4, m5, m7 = prod(0, 0), prod(1, 3), prod(2, 4), prod(3, 6)
        c11 = (m1 + m4) + (m7 - m5)
        m2, m3, m6 = prod(4, 1), prod(5, 2), prod(6, 5)
        c22 = (m1 - m2) + (m3 + m6)
        return jnp.concatenate([c11, m3 + m5], axis=1), jnp.concatenate([m2 + m4, c22], axis=1)

    for g in range(NGA):
        bdT = lax.dot_general(emat, wphi_ref[g * RA:(g + 1) * RA, :], NT_DIMS, preferred_element_type=f32)
        bd_s[g] = (bdT * bdm.astype(f32)).astype(bf16)

    def folded(part, g, it):
        w = kperm(sta_s[part * NGA + g, it * (L // 2):(it + 1) * (L // 2), :])
        return lax.dot_general(bd_s[g], w, NT_DIMS, preferred_element_type=f32) * LOG2E

    def put7(dst, it, quads, pinned):
        for i, w in enumerate(w_side(*quads)):
            w = pk(w)
            dst[i, :, it * L:(it + 1) * L] = w
            if pinned:
                pin(w)

    def prep_a(t, kv=True, q=True, its=range(4), pinned=False):
        for it in its:
            if kv:
                ts = jnp.minimum(t, NGA - 1) if not isinstance(t, int) else t
                vq = []
                for hf in range(2):
                    i2 = it + 4 * hf
                    vt = kperm(sta_s[2 * NGA + ts, i2 * (L // 2):(i2 + 1) * (L // 2), :]).astype(f32).T
                    for p in range(GA // 2):
                        for hh in range(2):
                            tmpa_s[i2, pl.ds(p * 64 + hh, DH, stride=2), :] = vt[p * 64 + hh * DH:p * 64 + (hh + 1) * DH]
                    vq.append(tmpa_s[i2])
                put7(wakv_s.at[t], it, [folded(1, ts, it), folded(1, ts, it + 4)] + vq, pinned)
            if q:
                q0, q1 = folded(0, t - 1, it), folded(0, t - 1, it + 4)
                put7(waq_s.at[t - 1], it, [q0[:64], q1[:64], q0[64:], q1[64:]], pinned)

    def prep_b(i, it, slot):
        rows = []
        for hf in range(2):
            i2 = it + 4 * hf
            tb = tmp_s.at[slot * (D // L) + i2]
            for half in range(2):
                wt = kperm(stb_s[i, half, i2 * (L // 2):(i2 + 1) * (L // 2), :]).astype(f32).T
                for u in range(16):
                    pos = ((u % 4) * 8 + half * 4 + u // 4) * 8
                    tb[pos:pos + 8, :] = wt[u * 8:u * 8 + 8]
            rows.append(jnp.concatenate([tb[pl.ds(64 * (d // 8) + d % 8, 8, stride=8), :] for d in range(DH)], axis=0))
        put7(wb_s.at[i], it, [rows[0][:L], rows[1][:L], rows[0][L:], rows[1][L:]], True)

    def prep_oa(g):
        cs = slice(g * RA, (g + 1) * RA)
        for ot in range(D // L):
            wo_p = jnp.dot(perm_o, stoa_s[cs, ot * L:(ot + 1) * L], preferred_element_type=f32)
            woa_s[ot * (L // 2):(ot + 1) * (L // 2), cs] = pk(wo_p.T)

    def prep_ob(g):
        for ot in range(D // L):
            tmpu_s[...] = pltpu.bitcast(stob_s[g * RB:(g + 1) * RB, ot * L:(ot + 1) * L], u32)
            rows = [tmpu_s[pl.ds(t, 8, stride=16), :] for t in range(16)]
            wr = upk(jnp.concatenate(rows, axis=0)).astype(f32)
            wob_s[ot * (L // 2):(ot + 1) * (L // 2), g * RB:g * RB + L] = pk(wr[0:L].T)
            wob_s[ot * (L // 2):(ot + 1) * (L // 2), g * RB + L:(g + 1) * RB] = pk(wr[L:2 * L].T)

    def xprep(jp):
        ssum = [None] * CT
        for dt in range(D // L):
            wt = xu_s[dt, pl.ds(jp, L, stride=NJ), :].T
            for c in range(CT):
                xc = pltpu.unpack_elementwise(wt, index=c, packed_dtype=bf16, unpacked_dtype=f32)
                xT_s[jp, dt * L:(dt + 1) * L, c * L:(c + 1) * L] = xc
                t = jnp.sum(xc.reshape(L // 8, 8, L), axis=0)
                ssum[c] = t if ssum[c] is None else ssum[c] + t
        _ln_finish(xT_s, hT_s, jp, jnp.concatenate(ssum, axis=1))

    kr = lax.broadcasted_iota(jnp.int32, (2 * DH, L), 0)
    kc = lax.broadcasted_iota(jnp.int32, (2 * DH, L), 1)
    par_mask = ((kr // 2) % 2) == (kc % 2)
    zr = lax.broadcasted_iota(jnp.int32, (16, L), 0)
    z_mask = (((zr // 2) % 2) == (lax.broadcasted_iota(jnp.int32, (16, L), 1) % 2)) & (zr < 8)

    def a_mm_kv(g, jp):
        kk, vv = smm(wakv_s.at[g], jp, NA_KV)
        buf = g % 2
        k_s[buf, jp, 0:RA, :] = kk
        vb_s[buf, jp] = pkf(vv)

    def a_mm_q(g, jp):
        q_s[jp, 0:RA, :] = jnp.concatenate(smm(waq_s.at[g], jp, NA_Q), axis=0)

    def a_phik(g, jp):
        buf = g % 2
        for p in range(GA // 2):
            phi = _phi_pair(k_s[buf, jp, p * 64:(p + 1) * 64, :])
            vv = upk(vb_s[buf, jp, p * DH:(p + 1) * DH, :])
            vaug = jnp.concatenate([vv, jnp.ones((16, NT), bf16)], axis=0)
            kv = lax.dot_general(vaug, phi, NT_DIMS, preferred_element_type=f32)
            if jp == 0:
                kvacc_s[p] = kv
            else:
                kvacc_s[p] += kv
            if TIEA: done(kv[0:8])

    def a_fin():
        for p in range(GA // 2):
            a = jnp.where(par_mask, kvacc_s[p, 0:2 * DH, :], 0.0)
            b = jnp.where(z_mask, kvacc_s[p, 2 * DH:, :], 0.0)
            kvT_s[p] = pk(jnp.concatenate([a, b], axis=0))

    def a_out(g, jp):
        for p in range(GA // 2):
            phi = _phi_pair(q_s[jp, p * 64:(p + 1) * 64, :])
            nd = jnp.dot(upk(kvT_s[p]), phi, preferred_element_type=f32)
            rcp = _rcp(tie(nd[2 * DH:2 * DH + 8]) + 1e-6)
            o = (nd[0:2 * DH].reshape(8, 8, NT) * rcp[None]).reshape(2 * DH, NT)
            ow = pkf(o)
            oT_s[jp, pl.ds(pl.multiple_of(g * (RA // 2) + p * DH, DH), DH), :] = ow
            if TIEA: done(ow)

    def layer_a(first):
        if first:
            for c in cps_a(0):
                c.wait()
            prep_a(0, q=False)
            with scope('xwait'):
                for dt in range(D // L):
                    cp_x(dt).wait()
            for t in range(1, NGA + 1):
                for c in cps_a(t):
                    c.start()
            for i in range(3 * NGB):
                cp_b(i, 0).start()
                cp_b(i, 1).start()
            cp_oa.start()
            cp_ob.start()
        for jp in range(NJ):
            if first:
                xprep(jp)
            a_mm_kv(0, jp)
            if first and jp == NJ // 2:
                for c in cps_a(1):
                    c.wait()
                prep_a(1)
        if first:
            for c in cps_a(2):
                c.wait()
            prep_a(2)
        for jp in range(NJ):
            a_mm_kv(1, jp)
            a_phik(0, jp)
        a_mm_q(0, 0)
        if first:
            for t in range(3, NGA + 1):
                for c in cps_a(t):
                    c.wait()

        def step_body(g, has_kv, last, prep):
            a_fin()
            if prep == 'loop':
                wait_b(2 * (g - 1))
                wait_b(2 * (g - 1) + 1)
            for jp in range(NJ):
                if has_kv:
                    a_mm_kv(g + 1, jp)
                if jp < NJ - 1:
                    a_mm_q(g - 1, jp + 1)
                elif not last:
                    a_mm_q(g, 0)
                if not last:
                    a_phik(g, jp)
                if prep == 'loop':
                    if jp % 2 == 0:
                        prep_a(g + 2, its=[jp // 2], pinned=True)
                    prep_b(2 * (g - 1) + jp % 2, jp // 2, jp % 2)
                elif prep is not None and jp % 2 == 0:
                    prep_oa(prep + jp // 2)
                a_out(g - 1, jp)

        def step(g, c):
            step_body(g, True, False, 'loop' if first else None)
            late.clear()
            return c
        late.clear()
        with scope('loopA'):
            lax.fori_loop(1, NGA - 1, step, 0)
        if first:
            cp_oa.wait()
        step_body(NGA - 1, False, False, 0 if first else None)
        step_body(NGA, False, True, 4 if first else None)

    lane0 = lax.broadcasted_iota(jnp.int32, (8, L), 1) == 0
    qscale = (DH ** -0.5) * LOG2E

    def b_mm_kv(g, jp):
        buf = g % 2
        for part, dst in ((0, k_s), (1, v_s)):
            r = jnp.concatenate(smm(wb_s.at[g * 3 + 1 + part], jp, NB_KV), axis=0)
            for c in range(CT):
                j = jp * CT + c
                kc = r[:, c * L:(c + 1) * L]
                dst[buf, (NC + j) // CT, :, c * L:(c + 1) * L] = kc
                if j >= 2:
                    dst[buf, jp, :, c * L:(c + 1) * L] = pltpu.roll(kc, 1, 1)

    def b_mm_q(g, jp):
        q_s[jp] = jnp.concatenate(smm(wb_s.at[g * 3], jp, NB_Q), axis=0) * qscale

    def b_att(g, jp):
        buf = g % 2
        for c in range(CT):
            j = jp * CT + c
            lanes = slice(c * L, (c + 1) * L)

            def win(ref, w, r0, r1):
                e = j - 2 * w + NC
                return ref[buf, e // CT, r0 * 8:r1 * 8, (e % CT) * L:(e % CT + 1) * L].reshape(r1 - r0, 8, L)

            if QKD == 0:
                q = q_s[jp, :, lanes].reshape(DH, 8, L)
                ls = []
                for w in range(W_WIN):
                    ls.append(jnp.sum(q * win(k_s, w, 0, DH), axis=0))
                    if w in QKW:
                        done(functools.reduce(jnp.maximum, ls))
            else:
                ls = [None] * W_WIN
                for r0, r1 in zip(QKW[:-1], QKW[1:]):
                    q = q_s[jp, r0 * 8:r1 * 8, lanes].reshape(r1 - r0, 8, L)
                    for w in range(W_WIN):
                        t = jnp.sum(q * win(k_s, w, r0, r1), axis=0)
                        ls[w] = t if ls[w] is None else ls[w] + t
                    if r1 < DH:
                        done(functools.reduce(jnp.maximum, ls))
            ls = [jnp.where(lane0, -1e9 * LOG2E, l) if 2 * w > j else l for w, l in enumerate(ls)]
            m = functools.reduce(jnp.maximum, ls)
            es = [jnp.exp2(l - m) for l in ls]
            rcp = _rcp(functools.reduce(lambda a, b: a + b, es))
            done(rcp)
            ps = [e_ * rcp for e_ in es]
            for r0, r1 in zip(PVW[:-1], PVW[1:]):
                acc = None
                for w in range(W_WIN):
                    t = win(v_s, w, r0, r1) * ps[w][None]
                    acc = t if acc is None else acc + t
                ow = pkf(acc.reshape((r1 - r0) * 8, L))
                oT_s[jp, pl.ds(pl.multiple_of(g * (RB // 2) + r0 * 4, 8), (r1 - r0) * 4), lanes] = ow
                done(ow)

    def layer_b():
        for jp in range(NJ):
            b_mm_kv(0, jp)
        b_mm_q(0, 0)

        def step_body(g, last):
            for jp in range(NJ):
                if ORDER == 1:
                    b_att(g, jp)
                if not last:
                    b_mm_kv(g + 1, jp)
                if jp < NJ - 1:
                    b_mm_q(g, jp + 1)
                elif not last:
                    b_mm_q(g + 1, 0)
                if ORDER == 1:
                    pass
                if last and KPRE:
                    for c in range(D // MC):
                        rs = slice(c * MC, (c + 1) * MC)
                        xT_s[jp, rs, :] += jnp.dot(upk(wob_s[c * (MC // 2):(c + 1) * (MC // 2), 0:KPRE]),
                                                   upk(oT_s[jp, 0:KPRE // 2, :]), preferred_element_type=f32)
                if ORDER == 0:
                    b_att(g, jp)

        def step(g, c):
            step_body(g, False)
            late.clear()
            return c
        late.clear()
        with scope('loopB'):
            lax.fori_loop(0, NGB - 1, step, 0)
        step_body(NGB - 1, True)

    def proj(wo_s, k0, prep=False):
        for jp in range(NJ):
            ssum = None
            for c in range(D // MC):
                rs = slice(c * MC, (c + 1) * MC)
                out = jnp.dot(upk(wo_s[c * (MC // 2):(c + 1) * (MC // 2), k0:]), upk(oT_s[jp, k0 // 2:, :]), preferred_element_type=f32)
                xn = xT_s[jp, rs, :] + out
                xT_s[jp, rs, :] = xn
                t = jnp.sum(xn.reshape(MC // 8, 8, NT), axis=0)
                ssum = t if ssum is None else ssum + t
            _ln_finish(xT_s, hT_s, jp, ssum)
            if prep and jp % 2 == 0:
                if jp == 0:
                    cp_ob.wait()
                prep_ob(jp // 2)

    def proj_last(wo_s, k0):
        for c in range(D // MC):
            rs = slice(c * MC, (c + 1) * MC)
            for jp in range(NJ):
                out = jnp.dot(upk(wo_s[c * (MC // 2):(c + 1) * (MC // 2), k0:]), upk(oT_s[jp, k0 // 2:, :]), preferred_element_type=f32)
                xn = xT_s[jp, rs, :] + out
                xu_s[c, pl.ds(jp, L, stride=NJ), :] = pltpu.pack_elementwise([xn[:, 0:L], xn[:, L:2 * L]], packed_dtype=bf16).T
            cp_out(c).start()
        with scope('owait'):
            for c in range(D // MC):
                cp_out(c).wait()

    if ONLY:
        for t in range(1, NGA + 1):
            for c in cps_a(t):
                c.start()
        for t in range(0, NGA + 1):
            for c in cps_a(t):
                c.wait()
        for dt in range(D // L):
            cp_x(dt).wait()
        lax.fori_loop(0, NJ, lambda jp, c: (xprep(jp), c)[1], 0)
        def fill(i, c):
            for it in range(8):
                blk = sta_s[8 + i, (it % 4) * L:(it % 4 + 1) * L, :]
                wob_s[pl.ds(pl.multiple_of((i % 4) * L, L), L), it * L:(it + 1) * L] = blk
                for q in range(2 if it < 4 else 0):
                    for z in range(7):
                        wb_s[i, z, :, it * L:(it + 1) * L] = blk[0:64]
                        wakv_s[i % 9, z, :, it * L:(it + 1) * L] = blk[0:64]
                        waq_s[i % 8, z, :, it * L:(it + 1) * L] = blk[0:32]
            return c
        lax.fori_loop(0, 12, fill, 0)
        if ONLY == 'B':
            layer_b()
            proj(wob_s, KPRE)
        else:
            layer_a(False)
            proj(wob_s, 0)
        for c in range(8):
            for z in range(4):
                xu_s[c, z * 256:(z + 1) * 256, :] = hT_s[c, z] | hT_s[c, z + 3]
            cp_out(c).start()
        for c in range(8):
            cp_out(c).wait()
        return
    layer_a(True)
    proj(woa_s, 0, True)
    layer_b()
    proj(wob_s, KPRE)
    layer_a(False)
    proj(woa_s, 0)
    layer_b()
    proj_last(wob_s, KPRE)


TIES = '1' == '1'
TIEA = '0' == '1'
FINE = int('0')
NB_KV, NB_Q, NA_KV, NA_Q = [int(v) for v in '4,4,0,0'.split(',')]
ONLY = ''
ORDER = int('0')
QKD = int('0')
QKW = [int(v) for v in '3'.split(',')]
PVW = [int(v) for v in '0,8,16,24,32'.split(',')]
SCOPES = False


def scope(name):
    import contextlib
    return jax.named_scope(name) if SCOPES else contextlib.nullcontext()


def build():
    hbm = pl.BlockSpec(memory_space=pl.ANY)
    vmem = pl.BlockSpec(memory_space=pltpu.VMEM)
    scratch = [
        pltpu.VMEM((D // L, S // 2, L), u32),
        pltpu.VMEM((3 * NGA, D // 2, RA), u32),
        pltpu.VMEM((3 * NGB, 2, D // 2, L), u32),
        pltpu.VMEM((D, D), bf16),
        pltpu.VMEM((D, D), bf16),
        pltpu.VMEM((NJ, D, NT), f32),
        pltpu.VMEM((NJ, 7, D // 4, L), u32),
        pltpu.VMEM((NJ, D // 2, NT), u32),
        pltpu.VMEM((NGA, 7, RA // 4, D // 2), u32),
        pltpu.VMEM((NGA + 1, 7, RA // 2, D // 2), u32),
        pltpu.VMEM((3 * NGB, 7, RB // 4, D // 2), u32),
        pltpu.VMEM((D // 2, D), u32),
        pltpu.VMEM((D // 2, D), u32),
        pltpu.VMEM((NGA, RA, RA), bf16),
        pltpu.VMEM((NJ, RB, NT), f32),
        pltpu.VMEM((2, 2 * NJ, RB, NT), f32),
        pltpu.VMEM((2, 2 * NJ, RB, NT), f32),
        pltpu.VMEM((2, NJ, RA // 2, NT), u32),
        pltpu.VMEM((GA // 2, 80, L), f32),
        pltpu.VMEM((GA // 2, 40, L), u32),
        pltpu.VMEM((2 * D // L, 2 * L, L), f32),
        pltpu.VMEM((D // L, L, L), f32),
        pltpu.VMEM((L, L), u32),
        pltpu.SemaphoreType.DMA((1,)),
        pltpu.SemaphoreType.DMA((4,)),
        pltpu.SemaphoreType.DMA((3 * NGB,)),
        pltpu.SemaphoreType.DMA((1,)),
        pltpu.SemaphoreType.DMA((1,)),
        pltpu.SemaphoreType.DMA((1,)),
    ]
    return pl.pallas_call(
        kernel,
        out_shape=jax.ShapeDtypeStruct((S, D), bf16),
        in_specs=[hbm, hbm, vmem, hbm, hbm, hbm, vmem],
        out_specs=hbm,
        scratch_shapes=scratch,
        compiler_params=pltpu.CompilerParams(vmem_limit_bytes=112 * 1024 * 1024),
    )


@jax.jit
def pallas_interleave_layers__linear_kernel_hedgehog__sliding_local_dilated__prompt_kernel(A_x, A_wqkv, A_w_phi, A_wo, B_x, B_wqkv, B_wo):
    cst = jnp.asarray(_consts(), bf16)
    out = build()(A_x.reshape(S, D), A_wqkv, A_w_phi.reshape(H * DH, DH), A_wo, B_wqkv, B_wo, cst)
    return out.reshape(1, S, D)
```

```python
import functools
import numpy as np
import jax
import jax.numpy as jnp
from jax import lax
from jax.experimental import pallas as pl
from jax.experimental.pallas import tpu as pltpu

S, D, H, DH = 2048, 1024, 32, 32
NC = 16
L = 128
GA = 4
NGA = H // GA
RA = GA * DH
GB = 8
NGB = H // GB
RB = GB * DH
CT = 2
NT = CT * L
NJ = NC // CT
W_WIN = 8
LOG2E = 1.4426950408889634
EPS = 1e-5
KPRE0 = 256
MC = 128
f32, bf16, u32 = jnp.float32, jnp.bfloat16, jnp.uint32
NT_DIMS = (((1,), (1,)), ((), ()))


def _sigma(k):
    return 16 * (k // 16) + 8 * (k % 2) + (k % 16) // 2


def _consts():
    def c_of_r(r):
        p, rr = r // 64, r % 64
        return p * 64 + (rr % 2) * 32 + rr // 2
    perm_v = np.zeros((RA, RA), np.float32)
    emat = np.zeros((RA, DH), np.float32)
    bdm = np.zeros((RA, RA), np.float32)
    perm_o = np.zeros((RA, RA), np.float32)
    for r in range(RA):
        c = c_of_r(r)
        perm_v[r, c] = 1
        emat[r, (r % 64) // 2] = 1
        bdm[r, (c // 32) * 32:(c // 32) * 32 + 32] = 1
    for k2 in range(RA):
        hf, p, kl = k2 // 64, (k2 % 64) // 32, k2 % 32
        perm_o[k2, c_of_r(p * 64 + _sigma(32 * hf + _sigma(kl)))] = 1
    return np.concatenate([bdm, perm_o, np.ones((16, RA), np.float32)], axis=0)


def pk(x):
    return pltpu.bitcast(x.astype(bf16), u32)


def pkf(x):
    n, m = x.shape[0] // 16, x.shape[1]
    x4 = x.reshape(n, 2, 8, m)
    return pltpu.pack_elementwise([x4[:, 0], x4[:, 1]], packed_dtype=bf16).reshape(8 * n, m)


def upk(x):
    return pltpu.bitcast(x, bf16)


def w_side(a11, a12, a21, a22):
    return [a11 + a22, a21 + a22, a11, a22, a11 + a12, a21 - a11, a12 - a22]


def h_side(b11, b12, b21, b22):
    return [b11 + b22, b11, b12 - b22, b21 - b11, b22, b11 + b12, b21 + b22]


def _rcp(x):
    return pl.reciprocal(x, approx=True)


def _par_all(x, op):
    x = op(x, pltpu.roll(x, 2, 0))
    return op(x, pltpu.roll(x, 4, 0))


def _sub_all(x):
    x = x + pltpu.roll(x, 1, 0)
    x = x + pltpu.roll(x, 2, 0)
    return x + pltpu.roll(x, 4, 0)


def _phi_pair(p):
    n = p.shape[1]
    p3 = p.reshape(8, 8, n)
    mx = _par_all(jnp.max(p3, axis=0), jnp.maximum)
    mn = _par_all(jnp.min(p3, axis=0), jnp.minimum)
    e1 = jnp.exp2(p3 - mx[None])
    e2 = jnp.exp2(mn[None] - p3)
    r1 = _rcp(_par_all(jnp.sum(e1, axis=0), jnp.add))
    r2 = _rcp(_par_all(jnp.sum(e2, axis=0), jnp.add))
    a = (e1 * r1[None]).reshape(2 * DH, n)
    b = (e2 * r2[None]).reshape(2 * DH, n)
    return jnp.concatenate([a, b], axis=0).astype(bf16)


def _ln_finish(xT_s, hT_s, jp, ssum, done=None):
    m = _sub_all(ssum) * (1.0 / D)
    acc = None
    for c in range(D // MC):
        d = xT_s[jp, c * MC:(c + 1) * MC, :].reshape(MC // 8, 8, NT) - m[None]
        t = jnp.sum(d * d, axis=0)
        acc = t if acc is None else acc + t
        if done and c % VP == VP - 1:
            done(acc)
    r = lax.rsqrt(_sub_all(acc) * (1.0 / D) + EPS)
    for c in range(D // 2 // MC):
        t, b = [((xT_s[jp, r0:r0 + MC, :].reshape(MC // 8, 8, NT) - m[None]) * r[None]).reshape(MC, NT)
                for r0 in (c * MC, D // 2 + c * MC)]
        for i, hh in enumerate(h_side(t[:, :L], t[:, L:], b[:, :L], b[:, L:])):
            hh = pkf(hh)
            hT_s[jp, i, c * (MC // 2):(c + 1) * (MC // 2), :] = hh
        if done:
            done(hh)


def kernel(x_hbm, awqkv_hbm, wphi_ref, awo_hbm, bwqkv_hbm, bwo_hbm, cst_ref, o_hbm,
           xu_s, sta_s, stb_s, stoa_s, stob_s,
           xT_s, hT_s, oT_s, waq_s, wakv_s, wb_s, woa_s, wob_s, bd_s,
           q_s, k_s, v_s, vb_s, kvacc_s, kvT_s, tmp_s, tmpa_s, tmpu_s, of_s, ss_s,
           sem_x, sem_a, sem_b, sem_oa, sem_ob, sem_o):
    def cp_x(dt):
        return pltpu.make_async_copy(x_hbm.at[:, pl.ds(dt * L, L)], xu_s.at[dt].bitcast(bf16), sem_x.at[dt])

    def cp_outs(dt):
        n = S // OSPL
        return [pltpu.make_async_copy(xu_s.at[dt, pl.ds(r * n // 2, n // 2)].bitcast(bf16),
                                      o_hbm.at[pl.ds(r * n, n), pl.ds(dt * L, L)], sem_o.at[0]) for r in range(OSPL)]

    def cp_a(part, g):
        t = g if part > 0 else g + 1
        return pltpu.make_async_copy(awqkv_hbm.at[:, pl.ds(part * D + g * RA, RA)],
                                     sta_s.at[part * NGA + g].bitcast(bf16), sem_a.at[min(t, 3)])

    def cps_a(t):
        return ([cp_a(1, t), cp_a(2, t)] if t < NGA else []) + ([cp_a(0, t - 1)] if t > 0 else [])

    def cp_b(i, half):
        g, part = i // 3, i % 3
        return pltpu.make_async_copy(bwqkv_hbm.at[:, pl.ds(part * D + g * RB + half * L, L)],
                                     stb_s.at[i, half].bitcast(bf16), sem_b.at[i])

    def wait_b(i):
        for half in range(2):
            pltpu.make_async_copy(bwqkv_hbm.at[:, pl.ds(0, L)], stb_s.at[i, half].bitcast(bf16), sem_b.at[i]).wait()

    cp_oa = pltpu.make_async_copy(awo_hbm, stoa_s, sem_oa.at[0])
    cp_ob = pltpu.make_async_copy(bwo_hbm, stob_s, sem_ob.at[0])

    for c in cps_a(0):
        c.start()
    for dt in range(NFLY):
        cp_x(dt).start()

    bdm = cst_ref[0:RA, :]
    perm_o = cst_ref[RA:2 * RA, :]
    e_r = lax.broadcasted_iota(jnp.int32, (RA, DH), 0)
    e_f = lax.broadcasted_iota(jnp.int32, (RA, DH), 1)
    emat = jnp.where((e_r % 64) // 2 == e_f, 1.0, 0.0).astype(bf16)

    def kperm(w):
        return upk(pkf(upk(w).astype(f32)))

    pins = []
    always = cst_ref[2 * RA:2 * RA + 16, :].astype(f32)[0:8] > 0.0

    def pin(words):
        words = words.astype(f32) if words.dtype == bf16 and PINF else words
        words = words if words.dtype == u32 else pltpu.bitcast(words, u32)
        pins.append(functools.reduce(jnp.bitwise_or, [words[i:i + 8, j:j + L] for i in range(0, words.shape[0], 8)
                                                      for j in range(0, words.shape[1], L)]))

    def tie(x):
        if not pins:
            return x
        junk = pltpu.bitcast(functools.reduce(jnp.bitwise_or, pins), f32)
        pins.clear()
        return jnp.concatenate([jnp.where(always, x[:, 0:L], junk), x[:, L:]], axis=1)

    late = []

    def done(words):
        words = words if words.dtype == u32 else pltpu.bitcast(words, u32)
        late.append(functools.reduce(jnp.bitwise_or, [words[i:i + 8, j:j + L] for i in range(0, words.shape[0], 8)
                                                      for j in range(0, words.shape[1], L)]))

    def patch(x, pts):
        if not pts:
            return x
        cols = []
        for c in range(x.shape[1] // L):
            rows, r = [], 0
            for (k, cc), junk in sorted(pts.items(), key=lambda kv: kv[0]):
                if cc == c:
                    if k > r:
                        rows.append(x[r:k, c * L:(c + 1) * L])
                    rows.append(jnp.where(always, x[k:k + 8, c * L:(c + 1) * L], junk))
                    r = k + 8
            if r < x.shape[0]:
                rows.append(x[r:, c * L:(c + 1) * L])
            cols.append(jnp.concatenate(rows, axis=0) if len(rows) > 1 else rows[0])
        return jnp.concatenate(cols, axis=1)

    def strassen(wget, hget, n=0):
        if not TIES:
            late.clear()
        n = min(n, 7, len(late))
        stops = {i * 7 // n: late.pop(0) for i in range(n)}

        def prod(pos, i):
            h = hget(i)
            if pos in stops:
                h = patch(h, {(0, 0): stops[pos]})
            return jnp.dot(upk(wget(i)), upk(h), preferred_element_type=f32)

        m1, m4, m5, m7 = prod(0, 0), prod(1, 3), prod(2, 4), prod(3, 6)
        c11 = (m1 + m4) + (m7 - m5)
        m2, m3, m6 = prod(4, 1), prod(5, 2), prod(6, 5)
        c22 = (m1 - m2) + (m3 + m6)
        return jnp.concatenate([c11, m3 + m5], axis=1), jnp.concatenate([m2 + m4, c22], axis=1)

    def smm(w, jp, n=0):
        w = w.bitcast(u32)
        return strassen(lambda i: jnp.concatenate([w[i, k] for k in range(4)], axis=1), lambda i: hT_s[jp, i], n)

    def omm(wo_s, jp, c, k0, k1, n=0):
        w = wo_s.at[c].bitcast(u32)
        return strassen(lambda i: jnp.concatenate([w[i, k] for k in range(k0 // L, k1 // L)], axis=1),
                        lambda i: oT_s[jp, i, k0 // 2:k1 // 2, :], n)

    for g in range(NGA):
        bdT = lax.dot_general(emat, wphi_ref[g * RA:(g + 1) * RA, :], NT_DIMS, preferred_element_type=f32)
        bd_s[g] = (bdT * bdm.astype(f32)).astype(bf16)

    def folded(part, g, it):
        w = kperm(sta_s[part * NGA + g, it * (L // 2):(it + 1) * (L // 2), :])
        return lax.dot_general(bd_s[g], w, NT_DIMS, preferred_element_type=f32) * LOG2E

    def put7(dst, it, quads, pinned):
        for i, w in enumerate(w_side(*quads)):
            w = w.astype(bf16)
            dst[i, it] = w
            if pinned:
                pinned(dst.bitcast(u32)[i, it])

    def prep_a(t, kv=True, q=True, its=range(4), pinned=False):
        for it in its:
            if kv:
                ts = jnp.minimum(t, NGA - 1) if not isinstance(t, int) else t
                vq = []
                for hf in range(2):
                    i2 = it + 4 * hf
                    vt = kperm(sta_s[2 * NGA + ts, i2 * (L // 2):(i2 + 1) * (L // 2), :]).astype(f32).T
                    for p in range(GA // 2):
                        for hh in range(2):
                            tmpa_s[i2, pl.ds(p * 64 + hh, DH, stride=2), :] = vt[p * 64 + hh * DH:p * 64 + (hh + 1) * DH]
                    vq.append(tmpa_s[i2])
                put7(wakv_s.at[t], it, [folded(1, ts, it), folded(1, ts, it + 4)] + vq, pinned)
            if q:
                q0, q1 = folded(0, t - 1, it), folded(0, t - 1, it + 4)
                put7(waq_s.at[t - 1], it, [q0[:64], q1[:64], q0[64:], q1[64:]], pinned)

    def prep_b(i, it, slot):
        rows = []
        for hf in range(2):
            i2 = it + 4 * hf
            tb = tmp_s.at[slot * (D // L) + i2]
            for half in range(2):
                wt = kperm(stb_s[i, half, i2 * (L // 2):(i2 + 1) * (L // 2), :]).astype(f32).T
                for u in range(16):
                    pos = ((u % 4) * 8 + half * 4 + u // 4) * 8
                    tb[pos:pos + 8, :] = wt[u * 8:u * 8 + 8]
            rows.append(jnp.concatenate([tb[pl.ds(64 * (d // 8) + d % 8, 8, stride=8), :] for d in range(DH)], axis=0))
        put7(wb_s.at[i], it, [rows[0][:L], rows[1][:L], rows[0][L:], rows[1][L:]], pin)

    def prep_oa(gp, c):
        quads = []
        for ot in (c, c + D // 2 // MC):
            for hf in range(2):
                pm = perm_o[hf * 64:(hf + 1) * 64]
                quads.append(jnp.concatenate(
                    [jnp.dot(pm, stoa_s[g * RA:(g + 1) * RA, ot * L:(ot + 1) * L], preferred_element_type=f32)
                     for g in (2 * gp, 2 * gp + 1)], axis=0).T)
        put7(woa_s.at[c], gp, quads, pin)

    def prep_ob(g, c):
        quads = []
        for n_, ot in enumerate((c, c + D // 2 // MC)):
            tb = tmpu_s.at[2 * c + n_]
            tb[...] = pltpu.bitcast(stob_s[g * RB:(g + 1) * RB, ot * L:(ot + 1) * L], u32)
            for hf in range(2):
                rows = [tb[pl.ds(t, 8, stride=16), :] for t in range(8 * hf, 8 * hf + 8)]
                quads.append(upk(jnp.concatenate(rows, axis=0)).astype(f32).T)
        put7(wob_s.at[c], g, quads, done)

    def xload(dt):
        for jp in range(NJ):
            wt = xu_s[dt, pl.ds(jp, L, stride=NJ), :].T
            xc = jnp.concatenate([pltpu.unpack_elementwise(wt, index=c, packed_dtype=bf16, unpacked_dtype=f32)
                                  for c in range(CT)], axis=1)
            xT_s[jp, dt * L:(dt + 1) * L, :] = xc
            t = jnp.sum(xc.reshape(L // 8, 8, NT), axis=0)
            ss_s[jp] = t if dt == 0 else ss_s[jp] + t

    def xprep(jp):
        _ln_finish(xT_s, hT_s, jp, ss_s[jp])

    kr = lax.broadcasted_iota(jnp.int32, (2 * DH, L), 0)
    kc = lax.broadcasted_iota(jnp.int32, (2 * DH, L), 1)
    par_mask = ((kr // 2) % 2) == (kc % 2)
    zr = lax.broadcasted_iota(jnp.int32, (16, L), 0)
    z_mask = (((zr // 2) % 2) == (lax.broadcasted_iota(jnp.int32, (16, L), 1) % 2)) & (zr < 8)

    def a_mm_kv(g, jp):
        kk, vv = smm(wakv_s.at[g], jp, NA_KV)
        buf = g % 2
        k_s[buf, jp, 0:RA, :] = kk
        vb_s[buf, jp] = pkf(vv)

    def a_mm_q(g, jp):
        q_s[jp, 0:RA, :] = jnp.concatenate(smm(waq_s.at[g], jp, NA_Q), axis=0)

    def a_phik(g, jp):
        buf = g % 2
        for p in range(GA // 2):
            phi = _phi_pair(k_s[buf, jp, p * 64:(p + 1) * 64, :])
            vv = upk(vb_s[buf, jp, p * DH:(p + 1) * DH, :])
            vaug = jnp.concatenate([vv, jnp.ones((16, NT), bf16)], axis=0)
            kv = lax.dot_general(vaug, phi, NT_DIMS, preferred_element_type=f32)
            if jp == 0:
                kvacc_s[p] = kv
            else:
                kvacc_s[p] += kv
            if TIEA: done(kv[0:8])

    def a_fin():
        for p in range(GA // 2):
            a = jnp.where(par_mask, kvacc_s[p, 0:2 * DH, :], 0.0)
            b = jnp.where(z_mask, kvacc_s[p, 2 * DH:, :], 0.0)
            kvT_s[p] = pk(jnp.concatenate([a, b], axis=0))

    def a_out(g, jp):
        for p in range(GA // 2):
            phi = _phi_pair(q_s[jp, p * 64:(p + 1) * 64, :])
            nd = jnp.dot(upk(kvT_s[p]), phi, preferred_element_type=f32)
            rcp = _rcp(tie(nd[2 * DH:2 * DH + 8]) + 1e-6)
            o = (nd[0:2 * DH].reshape(8, 8, NT) * rcp[None]).reshape(2 * DH, NT)
            for i, hh in enumerate(h_side(o[:DH, :L], o[:DH, L:], o[DH:, :L], o[DH:, L:])):
                oT_s[jp, i, pl.ds(pl.multiple_of(g * (RA // 4) + p * (DH // 2), DH // 2), DH // 2), :] = pkf(hh)

    def layer_a(first):
        if first:
            for c in cps_a(0):
                c.wait()
            prep_a(0, q=False)
            for dt in range(D // L):
                with scope('xwait'):
                    cp_x(dt).wait()
                if dt + NFLY < D // L:
                    cp_x(dt + NFLY).start()
                elif dt + NFLY == D // L + NFLY - 1:
                    for t in range(1, NGA + 1):
                        for c in cps_a(t):
                            c.start()
                xload(dt)
        for jp in range(NJ):
            if first:
                xprep(jp)
            a_mm_kv(0, jp)
            if first and jp == NJ // 2:
                for c in cps_a(1):
                    c.wait()
                prep_a(1)
        if first:
            for c in cps_a(2):
                c.wait()
            for i in range(3 * NGB):
                cp_b(i, 0).start()
                cp_b(i, 1).start()
            cp_oa.start()
            cp_ob.start()
            prep_a(2)
        for jp in range(NJ):
            a_mm_kv(1, jp)
            a_phik(0, jp)
        a_mm_q(0, 0)
        if first:
            for t in range(3, NGA + 1):
                for c in cps_a(t):
                    c.wait()

        def step_body(g, has_kv, last, prep):
            a_fin()
            if prep == 'loop':
                wait_b(2 * (g - 1))
                wait_b(2 * (g - 1) + 1)
            for jp in range(NJ):
                if has_kv:
                    a_mm_kv(g + 1, jp)
                if jp < NJ - 1:
                    a_mm_q(g - 1, jp + 1)
                elif not last:
                    a_mm_q(g, 0)
                if not last:
                    a_phik(g, jp)
                if prep == 'loop':
                    if jp % 2 == 0:
                        prep_a(g + 2, its=[jp // 2], pinned=pin)
                    prep_b(2 * (g - 1) + jp % 2, jp // 2, jp % 2)
                elif prep is not None:
                    prep_oa(prep + jp // 4, jp % 4)
                a_out(g - 1, jp)

        def step(g, c):
            step_body(g, True, False, 'loop' if first else None)
            late.clear()
            return c
        late.clear()
        with scope('loopA'):
            lax.fori_loop(1, NGA - 1, step, 0)
        if first:
            cp_oa.wait()
        step_body(NGA - 1, False, False, 0 if first else None)
        step_body(NGA, False, True, 2 if first else None)

    lane0 = lax.broadcasted_iota(jnp.int32, (8, L), 1) == 0
    qscale = (DH ** -0.5) * LOG2E

    def b_mm_kv(g, jp):
        buf = g % 2
        for part, dst in ((0, k_s), (1, v_s)):
            r = jnp.concatenate(smm(wb_s.at[g * 3 + 1 + part], jp, NB_KV), axis=0)
            for c in range(CT):
                j = jp * CT + c
                kc = r[:, c * L:(c + 1) * L]
                dst[buf, (NC + j) // CT, :, c * L:(c + 1) * L] = kc
                if j >= 2:
                    dst[buf, jp, :, c * L:(c + 1) * L] = pltpu.roll(kc, 1, 1)

    def b_mm_q(g, jp):
        q_s[jp] = jnp.concatenate(smm(wb_s.at[g * 3], jp, NB_Q), axis=0) * qscale

    def b_att(g, jp):
        buf = g % 2
        for c in range(CT):
            j = jp * CT + c
            lanes = slice(c * L, (c + 1) * L)

            def win(ref, w, r0, r1):
                e = j - 2 * w + NC
                return ref[buf, e // CT, r0 * 8:r1 * 8, (e % CT) * L:(e % CT + 1) * L].reshape(r1 - r0, 8, L)

            if QKD == 0:
                q = q_s[jp, :, lanes].reshape(DH, 8, L)
                ls = []
                for w in range(W_WIN):
                    ls.append(jnp.sum(q * win(k_s, w, 0, DH), axis=0))
                    if w in QKW:
                        done(functools.reduce(jnp.maximum, ls))
            else:
                ls = [None] * W_WIN
                for r0, r1 in zip(QKW[:-1], QKW[1:]):
                    q = q_s[jp, r0 * 8:r1 * 8, lanes].reshape(r1 - r0, 8, L)
                    for w in range(W_WIN):
                        t = jnp.sum(q * win(k_s, w, r0, r1), axis=0)
                        ls[w] = t if ls[w] is None else ls[w] + t
                    if r1 < DH:
                        done(functools.reduce(jnp.maximum, ls))
            ls = [jnp.where(lane0, -1e9 * LOG2E, l) if 2 * w > j else l for w, l in enumerate(ls)]
            m = functools.reduce(jnp.maximum, ls)
            es = [jnp.exp2(l - m) for l in ls]
            rcp = _rcp(functools.reduce(lambda a, b: a + b, es))
            done(rcp)
            ps = [e_ * rcp for e_ in es]
            def pv(r0, r1):
                acc = None
                for w in range(W_WIN):
                    t = win(v_s, w, r0, r1) * ps[w][None]
                    acc = t if acc is None else acc + t
                return acc.reshape((r1 - r0) * 8, L)

            for r0 in range(0, DH // 2, PVC):
                lo, hi = pv(r0, r0 + PVC), pv(DH // 2 + r0, DH // 2 + r0 + PVC)
                if c == 0:
                    of_s[r0 * 8:(r0 + PVC) * 8, :] = lo
                    of_s[RB // 2 + r0 * 8:RB // 2 + (r0 + PVC) * 8, :] = hi
                    done(lo)
                else:
                    for i, hh in enumerate(h_side(of_s[r0 * 8:(r0 + PVC) * 8, :], lo,
                                                  of_s[RB // 2 + r0 * 8:RB // 2 + (r0 + PVC) * 8, :], hi)):
                        ow = pkf(hh)
                        oT_s[jp, i, pl.ds(pl.multiple_of(g * (RB // 4) + r0 * 4, 8), PVC * 4), :] = ow
                    done(ow)

    def layer_b():
        for jp in range(NJ):
            b_mm_kv(0, jp)
        b_mm_q(0, 0)

        def step_body(g, last):
            for jp in range(NJ):
                if ORDER == 1:
                    b_att(g, jp)
                if not last:
                    b_mm_kv(g + 1, jp)
                if jp < NJ - 1:
                    b_mm_q(g, jp + 1)
                elif not last:
                    b_mm_q(g + 1, 0)
                if ORDER == 1:
                    pass
                if last and KPRE:
                    for c in range(D // 2 // MC):
                        for r0, part in zip((c * MC, D // 2 + c * MC), omm(wob_s, jp, c, 0, KPRE)):
                            xT_s[jp, r0:r0 + MC, :] += part
                if ORDER == 0:
                    b_att(g, jp)

        def step(g, c):
            step_body(g, False)
            late.clear()
            return c
        late.clear()
        with scope('loopB'):
            lax.fori_loop(0, NGB - 1, step, 0)
        step_body(NGB - 1, True)

    def proj(wo_s, k0, prep=False):
        for jp in range(NJ):
            ssum = None
            for c in range(D // 2 // MC):
                for r0, part in zip((c * MC, D // 2 + c * MC), omm(wo_s, jp, c, k0, D // 2, NP if prep else NL)):
                    xn = xT_s[jp, r0:r0 + MC, :] + part
                    xT_s[jp, r0:r0 + MC, :] = xn
                    t = jnp.sum(xn.reshape(MC // 8, 8, NT), axis=0)
                    ssum = t if ssum is None else ssum + t
            late.clear()
            _ln_finish(xT_s, hT_s, jp, ssum, done if LNT and not prep else None)
            if prep:
                if jp == 0:
                    cp_ob.wait()
                prep_ob(jp // 2, (jp % 2) * 2)
                prep_ob(jp // 2, (jp % 2) * 2 + 1)
        late.clear()

    def proj_last(wo_s, k0):
        for c in range(D // 2 // MC):
            for jp in range(NJ):
                for ot, part in zip((c, D // 2 // MC + c), omm(wo_s, jp, c, k0, D // 2)):
                    xn = xT_s[jp, ot * MC:(ot + 1) * MC, :] + part
                    xu_s[ot, pl.ds(jp, L, stride=NJ), :] = pltpu.pack_elementwise([xn[:, 0:L], xn[:, L:2 * L]], packed_dtype=bf16).T
            for cpo in cp_outs(c):
                cpo.start()
            for cpo in cp_outs(D // 2 // MC + c):
                cpo.start()
        with scope('owait'):
            for c in range(D // MC):
                for cpo in cp_outs(c):
                    cpo.wait()

    if ONLY:
        for t in range(1, NGA + 1):
            for c in cps_a(t):
                c.start()
        for t in range(0, NGA + 1):
            for c in cps_a(t):
                c.wait()
        for dt in range(NFLY, D // L):
            cp_x(dt).start()
        for dt in range(D // L):
            cp_x(dt).wait()
            xload(dt)
        lax.fori_loop(0, NJ, lambda jp, c: (xprep(jp), c)[1], 0)
        def fill(i, c):
            for it in range(4):
                blk = upk(sta_s[8 + i, it * 64:(it + 1) * 64, :])
                for z in range(7):
                    wob_s[i % 4, z, it] = blk
                    wb_s[i, z, it] = blk
                    wakv_s[i % 9, z, it] = blk
                    waq_s[i % 8, z, it] = blk[0:64]
            return c
        lax.fori_loop(0, 12, fill, 0)
        if ONLY == 'B':
            layer_b()
            proj(wob_s, KPRE)
        else:
            layer_a(False)
            proj(wob_s, 0)
        for c in range(8):
            for z in range(4):
                xu_s[c, z * 256:(z + 1) * 256, :] = hT_s[c, z] | hT_s[c, z + 3]
            for cpo in cp_outs(c):
                cpo.start()
        for c in range(8):
            for cpo in cp_outs(c):
                cpo.wait()
        return
    layer_a(True)
    proj(woa_s, 0, True)
    layer_b()
    proj(wob_s, KPRE)
    layer_a(False)
    proj(woa_s, 0)
    layer_b()
    proj_last(wob_s, KPRE)


TIES = '1' == '1'
TIEA = '0' == '1'
FINE = int('0')
NB_KV, NB_Q, NA_KV, NA_Q = [int(v) for v in '4,4,0,0'.split(',')]
ONLY = ''
ORDER = int('0')
QKD = int('0')
QKW = [int(v) for v in '3'.split(',')]
PVW = [int(v) for v in '0,8,16,24,32'.split(',')]
KPRE = int('128')
PVC = int('2')
NP = int('7')
PINF = 0
LNT = int('0')
XPOS = int('0')
FLAGS = {k: True for k in ''.split(',') if k} or None
NL = int('2')
VP = int('2')
NFLY = int('2')
OSPL = int('1')
SCOPES = False


def scope(name):
    import contextlib
    return jax.named_scope(name) if SCOPES else contextlib.nullcontext()


def build():
    hbm = pl.BlockSpec(memory_space=pl.ANY)
    vmem = pl.BlockSpec(memory_space=pltpu.VMEM)
    scratch = [
        pltpu.VMEM((D // L, S // 2, L), u32),
        pltpu.VMEM((3 * NGA, D // 2, RA), u32),
        pltpu.VMEM((3 * NGB, 2, D // 2, L), u32),
        pltpu.VMEM((D, D), bf16),
        pltpu.VMEM((D, D), bf16),
        pltpu.VMEM((NJ, D, NT), f32),
        pltpu.VMEM((NJ, 7, D // 4, L), u32),
        pltpu.VMEM((NJ, 7, D // 4, L), u32),
        pltpu.VMEM((NGA, 7, 4, RA // 2, L), bf16),
        pltpu.VMEM((NGA + 1, 7, 4, RA, L), bf16),
        pltpu.VMEM((3 * NGB, 7, 4, RB // 2, L), bf16),
        pltpu.VMEM((D // 2 // MC, 7, 4, MC, L), bf16),
        pltpu.VMEM((D // 2 // MC, 7, 4, MC, L), bf16),
        pltpu.VMEM((NGA, RA, RA), bf16),
        pltpu.VMEM((NJ, RB, NT), f32),
        pltpu.VMEM((2, 2 * NJ, RB, NT), f32),
        pltpu.VMEM((2, 2 * NJ, RB, NT), f32),
        pltpu.VMEM((2, NJ, RA // 2, NT), u32),
        pltpu.VMEM((GA // 2, 80, L), f32),
        pltpu.VMEM((GA // 2, 40, L), u32),
        pltpu.VMEM((2 * D // L, 2 * L, L), f32),
        pltpu.VMEM((D // L, L, L), f32),
        pltpu.VMEM((D // L, L, L), u32),
        pltpu.VMEM((RB, L), f32),
        pltpu.VMEM((NJ, 8, NT), f32),
        pltpu.SemaphoreType.DMA((D // L,)),
        pltpu.SemaphoreType.DMA((4,)),
        pltpu.SemaphoreType.DMA((3 * NGB,)),
        pltpu.SemaphoreType.DMA((1,)),
        pltpu.SemaphoreType.DMA((1,)),
        pltpu.SemaphoreType.DMA((1,)),
    ]
    return pl.pallas_call(
        kernel,
        out_shape=jax.ShapeDtypeStruct((S, D), bf16),
        in_specs=[hbm, hbm, vmem, hbm, hbm, hbm, vmem],
        out_specs=hbm,
        scratch_shapes=scratch,
        compiler_params=pltpu.CompilerParams(vmem_limit_bytes=112 * 1024 * 1024, flags=FLAGS),
    )


@jax.jit
def pallas_interleave_layers__linear_kernel_hedgehog__sliding_local_dilated__prompt_kernel(A_x, A_wqkv, A_w_phi, A_wo, B_x, B_wqkv, B_wo):
    cst = jnp.asarray(_consts(), bf16)
    out = build()(A_x.reshape(S, D), A_wqkv, A_w_phi.reshape(H * DH, DH), A_wo, B_wqkv, B_wo, cst)
    return out.reshape(1, S, D)
```
